```python
import jax
import jax.numpy as jnp

def _softmax(x, axis=-1):
    return jax.nn.softmax(x, axis=axis)
def _gelu(x):
    return jax.nn.gelu(x, approximate=True)
def _silu(x):
    return jax.nn.silu(x)
def _sigmoid(x):
    return jax.nn.sigmoid(x)
def _layernorm(x, axis=-1, eps=1e-5):
    m = jnp.mean(x, axis=axis, keepdims=True)
    v = jnp.var(x, axis=axis, keepdims=True)
    return (x - m) / jnp.sqrt(v + eps)
def _scatter_add(tgt, idx, src, axis=0):
    return tgt.at[idx].add(src)
def _segment_sum(src, seg, n):
    return jax.ops.segment_sum(src, seg, n)
class _Rng:
    def __init__(self, key):
        self._k = key
    def _next(self):
        self._k, sub = jax.random.split(self._k)
        return sub
    def normal(self, shape):
        return jax.random.normal(self._next(), shape, dtype=jnp.bfloat16)
    def randint(self, lo, hi, shape):
        return jax.random.randint(self._next(), shape, lo, hi, dtype=jnp.int32)
    def uniform(self, shape, lo=0.0, hi=1.0):
        return jax.random.uniform(self._next(), shape, jnp.bfloat16, lo, hi)
    def permutation(self, n):
        return jax.random.permutation(self._next(), n)


kernel_name = 'gated_mix__compressed_kv_cla__sliding_block_cached__decode'

def setup_inputs():
    _rng = _Rng(jax.random.key(int.from_bytes(__import__("os").urandom(4), "little")))
    _w = (lambda a: (lambda t: t.astype(jnp.bfloat16) if jnp.issubdtype(t.dtype, jnp.floating) else t)(jnp.asarray(a)))
    def _A_setup():
        B, H, Sq, Sk, D, M = 8, 32, 1, 4096, 128, 512
        Dc = 4 * D
        return {
            "x": _w((lambda *s: _rng.normal(s) * 0.05)(B, Sq, M)),
            "c_kv": _w((lambda *s: _rng.normal(s) * 0.05)(B, Sk, Dc)),
            "w_q": _w((lambda *s: _rng.normal(s) * 0.05)(M, H, D) * (M ** -0.5)),
            "w_uk": _w((lambda *s: _rng.normal(s) * 0.05)(Dc, H, D) * (Dc ** -0.5)),
            "w_uv": _w((lambda *s: _rng.normal(s) * 0.05)(Dc, H, D) * (Dc ** -0.5)),
            "w_o": _w((lambda *s: _rng.normal(s) * 0.05)(H, D, M) * ((H * D) ** -0.5)),
        }
    _A_in = _A_setup()

    def _B_setup():
        B, Sq, D = 8, 1, 512
        Hq, Hkv, Sk, Dh = 32, 8, 4096, 128
        assert Hq % Hkv == 0, (Hq, Hkv)
        return {
            "x": _w((lambda *s: _rng.normal(s) * 0.05)(B, Sq, D)),
            "k_cache": _w((lambda *s: _rng.normal(s) * 0.05)(B, Hkv, Sk, Dh)),
            "v_cache": _w((lambda *s: _rng.normal(s) * 0.05)(B, Hkv, Sk, Dh)),
            "wq": _w((lambda *s: _rng.normal(s) * 0.05)(D, Hq * Dh) * (D ** -0.5)),
            "wo": _w((lambda *s: _rng.normal(s) * 0.05)(Hq * Dh, D) * ((Hq * Dh) ** -0.5)),
        }
    _B_in = _B_setup()

    return {
        "A_x": _A_in["x"],
        "A_c_kv": _A_in["c_kv"],
        "A_w_q": _A_in["w_q"],
        "A_w_uk": _A_in["w_uk"],
        "A_w_uv": _A_in["w_uv"],
        "A_w_o": _A_in["w_o"],
        "B_x": _B_in["x"],
        "B_k_cache": _B_in["k_cache"],
        "B_v_cache": _B_in["v_cache"],
        "B_wq": _B_in["wq"],
        "B_wo": _B_in["wo"],
        "gate_w": _w((lambda *s: _rng.normal(s) * 0.05)(512)),
    }

def reference(A_x, A_c_kv, A_w_q, A_w_uk, A_w_uv, A_w_o, B_x, B_k_cache, B_v_cache, B_wq, B_wo, gate_w):
    def _A_ref(x, c_kv, w_q, w_uk, w_uv, w_o):
        B, Sq, M = x.shape[0], x.shape[1], x.shape[2]
        Sk = c_kv.shape[1]
        H, D = w_q.shape[1], w_q.shape[2]
        q = jnp.einsum("bqm,mhd->bhqd", x, w_q)
        k = jnp.einsum("bkc,chd->bhkd", c_kv, w_uk)
        v = jnp.einsum("bkc,chd->bhkd", c_kv, w_uv)
        scores = jnp.einsum("bhqd,bhkd->bhqk", q, k) * (D ** -0.5)
        off = Sk - Sq
        qi = jnp.arange(Sq)[:, None]
        kj = jnp.arange(Sk)[None, :]
        cmask = kj <= (qi + off)
        scores = jnp.where(cmask[None, None], scores, -1e9)
        p = _softmax(scores, axis=-1)
        ctx = jnp.einsum("bhqk,bhkd->bhqd", p, v)
        return jnp.einsum("bhqd,hdm->bqm", ctx, w_o)

    def _B_ref(x, k_cache, v_cache, wq, wo):
        B, Sq, D = x.shape
        Hq, Dh = 32, 128
        Hkv, Sk = k_cache.shape[1], k_cache.shape[2]
        W = min(4096, max(256, Sk // 4))
        rep = Hq // Hkv
        q = (lambda x, *d: x.transpose(*d))((x @ wq).reshape(B, Sq, Hq, Dh), 0, 2, 1, 3)
        k = jnp.repeat(k_cache[:, :, Sk - W:, :], rep, axis=1)
        v = jnp.repeat(v_cache[:, :, Sk - W:, :], rep, axis=1)
        scores = jnp.einsum("bhqd,bhkd->bhqk", q, k) * (Dh ** -0.5)
        p = _softmax(scores, axis=-1)
        o = jnp.einsum("bhqk,bhkd->bhqd", p, v)
        return (lambda x, *d: x.transpose(*d))(o, 0, 2, 1, 3).reshape(B, Sq, Hq * Dh) @ wo

    x = A_x
    g = _sigmoid((x * gate_w).sum(-1, keepdims=True))
    a = _A_ref(x, A_c_kv, A_w_q, A_w_uk, A_w_uv, A_w_o)
    b = _B_ref(x, B_k_cache, B_v_cache, B_wq, B_wo)
    return g * a + (1 - g) * b
```

```python
import math

import jax
import jax.numpy as jnp
from jax import lax
import jax.experimental.pallas as pl
import jax.experimental.pallas.tpu as pltpu

B = 8
H = 32
D = 128
M = 512
DC = 512
SK = 4096
HKV = 8
WIN = 1024
CK = 1024
LOG2E = math.log2(math.e)
F32 = jnp.float32
BF16 = jnp.bfloat16
NT = (((1,), (1,)), ((), ()))


def _head_pair(w_u32, j):
    w = w_u32[pl.ds(j, 512, stride=H // 2), :]
    lo = pltpu.bitcast(w << 16, F32).astype(BF16)
    hi = pltpu.bitcast(w & jnp.uint32(0xFFFF0000), F32).astype(BF16)
    return lo, hi


def _kernel(x_hbm, gw_hbm, c_hbm, wq_hbm, wuk_hbm, wuv_hbm, wo_hbm, k_hbm, v_hbm,
            bwq_hbm, bwo_hbm, o_ref,
            x_v, gw_v, wq_u32, wuk_u32, wuv_u32, wo_v, bwq_v, bwo_v, c_v, k_v, v_v,
            q_s, qabs_s, qb_s, ctxc_s, ob_s, sems, small_sems):

    def weight_copy(src, dst, rows, r, t):
        n = rows // 4
        return pltpu.make_async_copy(src.at[pl.ds(t * n, n)], dst.at[pl.ds(t * n, n)],
                                     sems.at[r % 2, t])

    def c_copy(b, r, t):
        return pltpu.make_async_copy(c_hbm.at[b, pl.ds(t * CK, CK)],
                                     c_v.at[r % 2, pl.ds(t * CK, CK)], sems.at[r % 2, t])

    def kv_copy(b, r, t):
        src, dst = (k_hbm, k_v) if t % 2 == 0 else (v_hbm, v_v)
        g0 = (t // 2) * (HKV // 2)
        return pltpu.make_async_copy(src.at[b, pl.ds(g0, HKV // 2), pl.ds(SK - WIN, WIN)],
                                     dst.at[r % 2, pl.ds(g0, HKV // 2)], sems.at[r % 2, t])

    R_WQ, R_WUK, R_C, R_BWQ = 0, 1, 2, 10
    R_WUV, R_KV, R_WO, R_BWO = 11, 12, 20, 21
    cp_wq = lambda t: weight_copy(wq_hbm, wq_u32.bitcast(BF16), M * H, R_WQ, t)
    cp_wuk = lambda t: weight_copy(wuk_hbm, wuk_u32.bitcast(BF16), DC * H, R_WUK, t)
    cp_bwq = lambda t: weight_copy(bwq_hbm, bwq_v, M, R_BWQ, t)
    cp_wuv = lambda t: weight_copy(wuv_hbm, wuv_u32.bitcast(BF16), DC * H, R_WUV, t)
    cp_wo = lambda t: weight_copy(wo_hbm, wo_v, H * D, R_WO, t)
    cp_bwo = lambda t: weight_copy(bwo_hbm, bwo_v, H * D, R_BWO, t)

    x_cp = pltpu.make_async_copy(x_hbm, x_v, small_sems.at[0])
    gw_cp = pltpu.make_async_copy(gw_hbm, gw_v, small_sems.at[1])
    x_cp.start()
    for t in range(4):
        cp_wq(t).start()
    gw_cp.start()

    for t in range(4):
        cp_wq(t).wait()
        cp_wuk(t).start()
    x_cp.wait()
    x = x_v[...]

    def q_body(j, _):
        for p, w in enumerate(_head_pair(wq_u32, j)):
            row = pl.multiple_of((2 * j + p) * B, B)
            q_s[pl.ds(row, B), :] = jnp.dot(x, w, preferred_element_type=F32)
        return _
    lax.fori_loop(0, H // 2, q_body, None)

    for t in range(4):
        cp_wuk(t).wait()
        c_copy(0, R_C, t).start()

    def qabs_body(j, _):
        for p, w in enumerate(_head_pair(wuk_u32, j)):
            row = pl.multiple_of((2 * j + p) * B, B)
            q = q_s[pl.ds(row, B), :].astype(BF16)
            qa = lax.dot_general(q, w, NT, preferred_element_type=F32)
            for i in range(DC // 128):
                qabs_s[i, pl.ds(row, B), :] = qa[:, i * 128:(i + 1) * 128]
        return _
    lax.fori_loop(0, H // 2, qabs_body, None)

    def c_round(b, _):
        r = R_C + b
        qa = jnp.concatenate(
            [qabs_s[i, pl.ds(b, H, stride=B), :] for i in range(DC // 128)], axis=1
        ).astype(BF16)
        for t in range(4):
            c_copy(b, r, t).wait()

            @pl.when(b < B - 1)
            def _():
                c_copy(b + 1, r + 1, t).start()

            @pl.when(b == B - 1)
            def _():
                cp_bwq(t).start()

            c = c_v[r % 2, pl.ds(t * CK, CK), :]
            s = lax.dot_general(qa, c, NT, preferred_element_type=F32) * (D ** -0.5 * LOG2E)
            m_blk = s.max(axis=1, keepdims=True)
            if t == 0:
                m = m_blk
                p = jnp.exp2(s - m)
                l = p.sum(axis=1, keepdims=True)
                acc = jnp.dot(p.astype(BF16), c, preferred_element_type=F32)
            else:
                m_new = jnp.maximum(m, m_blk)
                alpha = jnp.exp2(m - m_new)
                p = jnp.exp2(s - m_new)
                l = alpha * l + p.sum(axis=1, keepdims=True)
                acc = alpha * acc + jnp.dot(p.astype(BF16), c, preferred_element_type=F32)
                m = m_new
        ctx = acc / l
        for i in range(DC // 128):
            ctxc_s[i, pl.ds(b, H, stride=B), :] = ctx[:, i * 128:(i + 1) * 128]
        return _
    lax.fori_loop(0, B, c_round, None)

    for t in range(4):
        cp_bwq(t).wait()
        cp_wuv(t).start()
    qb = jnp.dot(x, bwq_v[...], preferred_element_type=F32)
    for h in range(H):
        qb_s[pl.ds(h * B, B), :] = qb[:, h * D:(h + 1) * D]

    for t in range(4):
        cp_wuv(t).wait()
        kv_copy(0, R_KV, t).start()

    def ctx_body(j, _):
        for p, w in enumerate(_head_pair(wuv_u32, j)):
            row = pl.multiple_of((2 * j + p) * B, B)
            cc = jnp.concatenate(
                [ctxc_s[i, pl.ds(row, B), :] for i in range(DC // 128)], axis=1
            ).astype(BF16)
            q_s[pl.ds(row, B), :] = jnp.dot(cc, w, preferred_element_type=F32)
        return _
    lax.fori_loop(0, H // 2, ctx_body, None)

    def kv_round(b, _):
        r = R_KV + b
        for half in range(2):
            for t in (2 * half, 2 * half + 1):
                kv_copy(b, r, t).wait()

                @pl.when(b < B - 1)
                def _():
                    kv_copy(b + 1, r + 1, t).start()

                @pl.when(b == B - 1)
                def _():
                    cp_wo(t).start()

            for i in (2 * half, 2 * half + 1):
                q8 = qb_s[pl.ds(b + 8 * i * B, 8, stride=B), :].astype(BF16)
                first = lax.broadcasted_iota(jnp.int32, (8, 1), 0) < 4
                s0 = lax.dot_general(q8, k_v[r % 2, 2 * i], NT, preferred_element_type=F32)
                s1 = lax.dot_general(q8, k_v[r % 2, 2 * i + 1], NT, preferred_element_type=F32)
                s = jnp.where(first, s0, s1) * (D ** -0.5 * LOG2E)
                p = jnp.exp2(s - s.max(axis=1, keepdims=True))
                l = p.sum(axis=1, keepdims=True)
                pb = p.astype(BF16)
                o0 = jnp.dot(pb, v_v[r % 2, 2 * i], preferred_element_type=F32)
                o1 = jnp.dot(pb, v_v[r % 2, 2 * i + 1], preferred_element_type=F32)
                ob_s[pl.ds(b + 8 * i * B, 8, stride=B), :] = jnp.where(first, o0, o1) / l
        return _
    lax.fori_loop(0, B, kv_round, None)

    gw_cp.wait()
    gate = jax.nn.sigmoid(
        (x.astype(F32) * gw_v[...].astype(F32).reshape(1, M)).sum(axis=1, keepdims=True))

    def lhs(scratch, t):
        return jnp.concatenate(
            [scratch[pl.ds((8 * t + h) * B, B), :] for h in range(8)], axis=1).astype(BF16)

    out_a = jnp.zeros((B, M), F32)
    for t in range(4):
        cp_wo(t).wait()
        cp_bwo(t).start()
        out_a += jnp.dot(lhs(q_s, t), wo_v[pl.ds(t * 1024, 1024), :], preferred_element_type=F32)
    out = gate * out_a
    for t in range(4):
        ob = lhs(ob_s, t)
        cp_bwo(t).wait()
        out_b = jnp.dot(ob, bwo_v[pl.ds(t * 1024, 1024), :], preferred_element_type=F32)
        out += (1.0 - gate) * out_b
    o_ref[...] = out.astype(o_ref.dtype)


@jax.jit
def pallas_gated_mix__compressed_kv_cla__sliding_block_cached__decode_kernel(
    A_x: jax.Array,
    A_c_kv: jax.Array,
    A_w_q: jax.Array,
    A_w_uk: jax.Array,
    A_w_uv: jax.Array,
    A_w_o: jax.Array,
    B_x: jax.Array,
    B_k_cache: jax.Array,
    B_v_cache: jax.Array,
    B_wq: jax.Array,
    B_wo: jax.Array,
    gate_w: jax.Array,
):
    del B_x
    hbm = pl.BlockSpec(memory_space=pl.ANY)
    rows_bh = B * H
    out = pl.pallas_call(
        _kernel,
        out_shape=jax.ShapeDtypeStruct((B, M), BF16),
        in_specs=[hbm] * 11,
        out_specs=pl.BlockSpec(memory_space=pltpu.VMEM),
        scratch_shapes=[
            pltpu.VMEM((B, M), BF16),
            pltpu.VMEM((M,), BF16),
            pltpu.VMEM((M * H // 2, D), jnp.uint32),
            pltpu.VMEM((DC * H // 2, D), jnp.uint32),
            pltpu.VMEM((DC * H // 2, D), jnp.uint32),
            pltpu.VMEM((H * D, M), BF16),
            pltpu.VMEM((M, H * D), BF16),
            pltpu.VMEM((H * D, M), BF16),
            pltpu.VMEM((2, SK, DC), BF16),
            pltpu.VMEM((2, HKV, WIN, D), BF16),
            pltpu.VMEM((2, HKV, WIN, D), BF16),
            pltpu.VMEM((rows_bh, D), F32),
            pltpu.VMEM((DC // 128, rows_bh, 128), F32),
            pltpu.VMEM((rows_bh, D), F32),
            pltpu.VMEM((DC // 128, rows_bh, 128), F32),
            pltpu.VMEM((rows_bh, D), F32),
            pltpu.SemaphoreType.DMA((2, 4)),
            pltpu.SemaphoreType.DMA((2,)),
        ],
        compiler_params=pltpu.CompilerParams(vmem_limit_bytes=64 * 1024 * 1024),
    )(
        A_x.reshape(B, M), gate_w, A_c_kv,
        A_w_q.reshape(M * H, D), A_w_uk.reshape(DC * H, D), A_w_uv.reshape(DC * H, D),
        A_w_o.reshape(H * D, M), B_k_cache, B_v_cache, B_wq, B_wo,
    )
    return out.reshape(B, 1, M)
```

```python
import math

import jax
import jax.numpy as jnp
from jax import lax
import jax.experimental.pallas as pl
import jax.experimental.pallas.tpu as pltpu

B = 8
H = 32
D = 128
M = 512
DC = 512
SK = 4096
HKV = 8
WIN = 1024
CK = 1024
LOG2E = math.log2(math.e)
F32 = jnp.float32
BF16 = jnp.bfloat16

PIECE_BYTES = 32 * 1024
PATTERN = (0, 1)
NT = (((1,), (1,)), ((), ()))


def _head_pair(w_u32, t, j):
    w = w_u32[pl.ds(t * (128 * H // 2) + j, 128, stride=H // 2), :]
    lo = pltpu.bitcast(w << 16, F32).astype(BF16)
    hi = pltpu.bitcast(w & jnp.uint32(0xFFFF0000), F32).astype(BF16)
    return lo, hi


def _kernel(x_hbm, gw_hbm, c_hbm, wq_hbm, wuk_hbm, wuv_hbm, wo_hbm, k_hbm, v_hbm,
            bwq_hbm, bwo_hbm, o_ref,
            x_v, gw_v, wq_u32, wuk_u32, wuv_u32, wo_v, bwq_v, bwo_v, c_v, k_v, v_v,
            x_s, q_s, ctx_s, qabs_s, qb_s, ctxc_s, ob_s, sems, small_sems):

    class Chunk:
        def __init__(self, src, dst, sem, pieces):
            self.src, self.dst, self.sem, self.pieces = src, dst, sem, pieces

        def start(self):
            for n, idx in enumerate(self.pieces):
                pltpu.make_async_copy(self.src.at[idx], self.dst.at[idx], self.sem).start(
                    priority=PATTERN[n % len(PATTERN)])

        def wait(self):
            pltpu.make_async_copy(self.dst, self.dst, self.sem).wait()

    def row_pieces(rows, row_bytes):
        n = PIECE_BYTES // row_bytes
        return [(pl.ds(i * n, n),) for i in range(rows // n)]

    def weight_chunk(src, dst, rows, cols, r, t):
        n = rows // 4
        if cols * 2 * 8 > PIECE_BYTES:
            w = PIECE_BYTES // 16
            pieces = [(pl.ds(i * 8, 8), pl.ds(j * w, w)) for i in range(n // 8) for j in range(cols // w)]
        else:
            pieces = row_pieces(n, cols * 2)
        return Chunk(src.at[pl.ds(t * n, n)], dst.at[pl.ds(t * n, n)], sems.at[r % 2, t], pieces)

    def c_copy(b, r, t):
        return Chunk(c_hbm.at[b, pl.ds(t * CK, CK)], c_v.at[r % 2, pl.ds(t * CK, CK)],
                     sems.at[r % 2, t], row_pieces(CK, DC * 2))

    def kv_copy(b, r, t):
        src, dst = (k_hbm, k_v) if t % 2 == 0 else (v_hbm, v_v)
        g0 = (t // 2) * (HKV // 2)
        pieces = [(g,) + i for g in range(HKV // 2) for i in row_pieces(WIN, D * 2)]
        return Chunk(src.at[b, pl.ds(g0, HKV // 2), pl.ds(SK - WIN, WIN)],
                     dst.at[r % 2, pl.ds(g0, HKV // 2)], sems.at[r % 2, t], pieces)

    R_WQ, R_WUK, R_C, R_BWQ = 0, 1, 2, 10
    R_WUV, R_KV, R_WO, R_BWO = 11, 12, 20, 21
    cp_wq = lambda t: weight_chunk(wq_hbm, wq_u32.bitcast(BF16), M * H, D, R_WQ, t)
    cp_wuk = lambda t: weight_chunk(wuk_hbm, wuk_u32.bitcast(BF16), DC * H, D, R_WUK, t)
    cp_bwq = lambda t: weight_chunk(bwq_hbm, bwq_v, M, H * D, R_BWQ, t)
    cp_wuv = lambda t: weight_chunk(wuv_hbm, wuv_u32.bitcast(BF16), DC * H, D, R_WUV, t)
    cp_wo = lambda t: weight_chunk(wo_hbm, wo_v, H * D, M, R_WO, t)
    cp_bwo = lambda t: weight_chunk(bwo_hbm, bwo_v, H * D, M, R_BWO, t)

    x_cp = pltpu.make_async_copy(x_hbm, x_v, small_sems.at[0])
    gw_cp = pltpu.make_async_copy(gw_hbm, gw_v, small_sems.at[1])
    cp_wq(0).start()
    x_cp.start()
    for t in range(1, 4):
        cp_wq(t).start()
    gw_cp.start()

    x_cp.wait()
    x = x_v[...]
    for t in range(4):
        x_s[t] = x[:, t * 128:(t + 1) * 128].astype(F32)
    q_s[...] = jnp.zeros_like(q_s)
    ctx_s[...] = jnp.zeros_like(ctx_s)

    def q_step(t, _):
        cp_wq(t).wait()
        cp_wuk(t).start()
        xt = x_s[t].astype(BF16)
        for j in range(H // 2):
            for p, w in enumerate(_head_pair(wq_u32, t, j)):
                rows = pl.ds((2 * j + p) * B, B)
                q_s[rows, :] += jnp.dot(xt, w, preferred_element_type=F32)
        return _
    lax.fori_loop(0, 4, q_step, None)

    def qabs_step(t, _):
        cp_wuk(t).wait()
        c_copy(0, R_C, t).start()
        for j in range(H // 2):
            for p, w in enumerate(_head_pair(wuk_u32, t, j)):
                rows = pl.ds((2 * j + p) * B, B)
                q = q_s[rows, :].astype(BF16)
                qabs_s[t, rows, :] = lax.dot_general(q, w, NT, preferred_element_type=F32)
        return _
    lax.fori_loop(0, 4, qabs_step, None)

    def c_round(b, _):
        r = R_C + b
        qa = jnp.concatenate(
            [qabs_s[i, pl.ds(b, H, stride=B), :] for i in range(DC // 128)], axis=1
        ).astype(BF16)
        for t in range(4):
            c_copy(b, r, t).wait()

            @pl.when(b < B - 1)
            def _():
                c_copy(b + 1, r + 1, t).start()

            @pl.when(b == B - 1)
            def _():
                cp_bwq(t).start()

            c = c_v[r % 2, pl.ds(t * CK, CK), :]
            s = lax.dot_general(qa, c, NT, preferred_element_type=F32) * (D ** -0.5 * LOG2E)
            m_blk = s.max(axis=1, keepdims=True)
            if t == 0:
                m = m_blk
                p = jnp.exp2(s - m)
                l = p.sum(axis=1, keepdims=True)
                acc = jnp.dot(p.astype(BF16), c, preferred_element_type=F32)
            else:
                m_new = jnp.maximum(m, m_blk)
                alpha = jnp.exp2(m - m_new)
                p = jnp.exp2(s - m_new)
                l = alpha * l + p.sum(axis=1, keepdims=True)
                acc = alpha * acc + jnp.dot(p.astype(BF16), c, preferred_element_type=F32)
                m = m_new
        ctx = acc / l
        for i in range(DC // 128):
            ctxc_s[i, pl.ds(b, H, stride=B), :] = ctx[:, i * 128:(i + 1) * 128]
        return _
    lax.fori_loop(0, B, c_round, None)

    qb = None
    for t in range(4):
        cp_bwq(t).wait()
        cp_wuv(t).start()
        part = jnp.dot(x_s[t].astype(BF16), bwq_v[pl.ds(t * 128, 128), :], preferred_element_type=F32)
        qb = part if qb is None else qb + part
    for h in range(H):
        qb_s[pl.ds(h * B, B), :] = qb[:, h * D:(h + 1) * D]

    def ctx_step(t, _):
        cp_wuv(t).wait()
        for u in range(4):
            @pl.when(t == u)
            def _():
                kv_copy(0, R_KV, u).start()
        for j in range(H // 2):
            for p, w in enumerate(_head_pair(wuv_u32, t, j)):
                rows = pl.ds((2 * j + p) * B, B)
                cc = ctxc_s[t, rows, :].astype(BF16)
                ctx_s[rows, :] += jnp.dot(cc, w, preferred_element_type=F32)
        return _
    lax.fori_loop(0, 4, ctx_step, None)

    def kv_round(b, _):
        r = R_KV + b
        for half in range(2):
            for t in (2 * half, 2 * half + 1):
                kv_copy(b, r, t).wait()

                @pl.when(b < B - 1)
                def _():
                    kv_copy(b + 1, r + 1, t).start()

                @pl.when(b == B - 1)
                def _():
                    cp_wo(t).start()

            for i in (2 * half, 2 * half + 1):
                q8 = qb_s[pl.ds(b + 8 * i * B, 8, stride=B), :].astype(BF16)
                first = lax.broadcasted_iota(jnp.int32, (8, 1), 0) < 4
                s0 = lax.dot_general(q8, k_v[r % 2, 2 * i], NT, preferred_element_type=F32)
                s1 = lax.dot_general(q8, k_v[r % 2, 2 * i + 1], NT, preferred_element_type=F32)
                s = jnp.where(first, s0, s1) * (D ** -0.5 * LOG2E)
                p = jnp.exp2(s - s.max(axis=1, keepdims=True))
                l = p.sum(axis=1, keepdims=True)
                pb = p.astype(BF16)
                o0 = jnp.dot(pb, v_v[r % 2, 2 * i], preferred_element_type=F32)
                o1 = jnp.dot(pb, v_v[r % 2, 2 * i + 1], preferred_element_type=F32)
                ob_s[pl.ds(b + 8 * i * B, 8, stride=B), :] = jnp.where(first, o0, o1) / l
        return _
    lax.fori_loop(0, B, kv_round, None)

    gw_cp.wait()
    gate = jax.nn.sigmoid(
        (x.astype(F32) * gw_v[...].astype(F32).reshape(1, M)).sum(axis=1, keepdims=True))

    def lhs(scratch, t):
        return jnp.concatenate(
            [scratch[pl.ds((8 * t + h) * B, B), :] for h in range(8)], axis=1).astype(BF16)

    out_a = jnp.zeros((B, M), F32)
    for t in range(4):
        cp_wo(t).wait()
        cp_bwo(t).start()
        out_a += jnp.dot(lhs(ctx_s, t), wo_v[pl.ds(t * 1024, 1024), :], preferred_element_type=F32)
    out = gate * out_a
    for t in range(4):
        ob = lhs(ob_s, t)
        cp_bwo(t).wait()
        out_b = jnp.dot(ob, bwo_v[pl.ds(t * 1024, 1024), :], preferred_element_type=F32)
        out += (1.0 - gate) * out_b
    o_ref[...] = out.astype(o_ref.dtype)


@jax.jit
def pallas_gated_mix__compressed_kv_cla__sliding_block_cached__decode_kernel(
    A_x: jax.Array,
    A_c_kv: jax.Array,
    A_w_q: jax.Array,
    A_w_uk: jax.Array,
    A_w_uv: jax.Array,
    A_w_o: jax.Array,
    B_x: jax.Array,
    B_k_cache: jax.Array,
    B_v_cache: jax.Array,
    B_wq: jax.Array,
    B_wo: jax.Array,
    gate_w: jax.Array,
):
    del B_x
    hbm = pl.BlockSpec(memory_space=pl.ANY)
    rows_bh = B * H
    out = pl.pallas_call(
        _kernel,
        out_shape=jax.ShapeDtypeStruct((B, M), BF16),
        in_specs=[hbm] * 11,
        out_specs=pl.BlockSpec(memory_space=pltpu.VMEM),
        scratch_shapes=[
            pltpu.VMEM((B, M), BF16),
            pltpu.VMEM((M,), BF16),
            pltpu.VMEM((M * H // 2, D), jnp.uint32),
            pltpu.VMEM((DC * H // 2, D), jnp.uint32),
            pltpu.VMEM((DC * H // 2, D), jnp.uint32),
            pltpu.VMEM((H * D, M), BF16),
            pltpu.VMEM((M, H * D), BF16),
            pltpu.VMEM((H * D, M), BF16),
            pltpu.VMEM((2, SK, DC), BF16),
            pltpu.VMEM((2, HKV, WIN, D), BF16),
            pltpu.VMEM((2, HKV, WIN, D), BF16),
            pltpu.VMEM((4, B, 128), F32),
            pltpu.VMEM((rows_bh, D), F32),
            pltpu.VMEM((rows_bh, D), F32),
            pltpu.VMEM((DC // 128, rows_bh, 128), F32),
            pltpu.VMEM((rows_bh, D), F32),
            pltpu.VMEM((DC // 128, rows_bh, 128), F32),
            pltpu.VMEM((rows_bh, D), F32),
            pltpu.SemaphoreType.DMA((2, 4)),
            pltpu.SemaphoreType.DMA((2,)),
        ],
        compiler_params=pltpu.CompilerParams(vmem_limit_bytes=64 * 1024 * 1024),
    )(
        A_x.reshape(B, M), gate_w, A_c_kv,
        A_w_q.reshape(M * H, D), A_w_uk.reshape(DC * H, D), A_w_uv.reshape(DC * H, D),
        A_w_o.reshape(H * D, M), B_k_cache, B_v_cache, B_wq, B_wo,
    )
    return out.reshape(B, 1, M)
```

```python
import math

import jax
import jax.numpy as jnp
from jax import lax
import jax.experimental.pallas as pl
import jax.experimental.pallas.tpu as pltpu

B = 8
H = 32
D = 128
M = 512
DC = 512
SK = 4096
HKV = 8
WIN = 1024
CK = 1024
LOG2E = math.log2(math.e)
F32 = jnp.float32
BF16 = jnp.bfloat16

PIECE_BYTES = 32 * 1024
SPLIT = True
PATTERN = (0, 1)
NT = (((1,), (1,)), ((), ()))


def _head_pair(w_u32, t, j):
    w = w_u32[pl.ds(t * (128 * H // 2) + j, 128, stride=H // 2), :]
    lo = pltpu.bitcast(w << 16, F32).astype(BF16)
    hi = pltpu.bitcast(w & jnp.uint32(0xFFFF0000), F32).astype(BF16)
    return lo, hi


def _kernel(x_hbm, gw_hbm, c_hbm, wq_hbm, wuk_hbm, wuv_hbm, wo_hbm, k_hbm, v_hbm,
            bwq_hbm, bwo_hbm, o_ref,
            x_v, gw_v, wq_u32, wuk_u32, wuv_u32, wo_v, bwq_v, bwo_v, c_v, k_v, v_v,
            x_s, q_s, ctx_s, qabs_s, qb_s, ctxc_s, ob_s, sems, small_sems):

    class Chunk:
        def __init__(self, src, dst, sem, pieces):
            self.src, self.dst, self.sem, self.pieces = src, dst, sem, pieces

        def start(self):
            half = len(self.pieces) // 2
            for n in range(len(self.pieces)):
                idx = self.pieces[n // 2 + (n % 2) * half] if SPLIT else self.pieces[n]
                pltpu.make_async_copy(self.src.at[idx], self.dst.at[idx], self.sem).start(
                    priority=PATTERN[n % len(PATTERN)])

        def wait(self):
            pltpu.make_async_copy(self.dst, self.dst, self.sem).wait()

    def row_pieces(rows, row_bytes):
        n = PIECE_BYTES // row_bytes
        return [(pl.ds(i * n, n),) for i in range(rows // n)]

    def weight_chunk(src, dst, rows, cols, r, t):
        n = rows // 4
        if cols * 2 * 8 > PIECE_BYTES:
            w = PIECE_BYTES // 16
            pieces = [(pl.ds(i * 8, 8), pl.ds(j * w, w)) for i in range(n // 8) for j in range(cols // w)]
        else:
            pieces = row_pieces(n, cols * 2)
        return Chunk(src.at[pl.ds(t * n, n)], dst.at[pl.ds(t * n, n)], sems.at[r % 2, t], pieces)

    def c_copy(b, r, t):
        return Chunk(c_hbm.at[b, pl.ds(t * CK, CK)], c_v.at[r % 2, pl.ds(t * CK, CK)],
                     sems.at[r % 2, t], row_pieces(CK, DC * 2))

    def kv_copy(b, r, t):
        src, dst = (k_hbm, k_v) if t % 2 == 0 else (v_hbm, v_v)
        g0 = (t // 2) * (HKV // 2)
        pieces = [(g,) + i for g in range(HKV // 2) for i in row_pieces(WIN, D * 2)]
        return Chunk(src.at[b, pl.ds(g0, HKV // 2), pl.ds(SK - WIN, WIN)],
                     dst.at[r % 2, pl.ds(g0, HKV // 2)], sems.at[r % 2, t], pieces)

    R_WQ, R_WUK, R_C, R_BWQ = 0, 1, 2, 10
    R_WUV, R_KV, R_WO, R_BWO = 11, 12, 20, 21
    cp_wq = lambda t: weight_chunk(wq_hbm, wq_u32.bitcast(BF16), M * H, D, R_WQ, t)
    cp_wuk = lambda t: weight_chunk(wuk_hbm, wuk_u32.bitcast(BF16), DC * H, D, R_WUK, t)
    cp_bwq = lambda t: weight_chunk(bwq_hbm, bwq_v, M, H * D, R_BWQ, t)
    cp_wuv = lambda t: weight_chunk(wuv_hbm, wuv_u32.bitcast(BF16), DC * H, D, R_WUV, t)
    cp_wo = lambda t: weight_chunk(wo_hbm, wo_v, H * D, M, R_WO, t)
    cp_bwo = lambda t: weight_chunk(bwo_hbm, bwo_v, H * D, M, R_BWO, t)

    x_cp = pltpu.make_async_copy(x_hbm, x_v, small_sems.at[0])
    gw_cp = pltpu.make_async_copy(gw_hbm, gw_v, small_sems.at[1])
    cp_wq(0).start()
    x_cp.start()
    for t in range(1, 4):
        cp_wq(t).start()
    gw_cp.start()

    x_cp.wait()
    x = x_v[...]
    for t in range(4):
        x_s[t] = x[:, t * 128:(t + 1) * 128].astype(F32)
    q_s[...] = jnp.zeros_like(q_s)
    ctx_s[...] = jnp.zeros_like(ctx_s)

    def q_step(t, _):
        cp_wq(t).wait()
        cp_wuk(t).start()
        xt = x_s[t].astype(BF16)
        for j in range(H // 2):
            for p, w in enumerate(_head_pair(wq_u32, t, j)):
                rows = pl.ds((2 * j + p) * B, B)
                q_s[rows, :] += jnp.dot(xt, w, preferred_element_type=F32)
        return _
    lax.fori_loop(0, 4, q_step, None)

    def qabs_step(t, _):
        cp_wuk(t).wait()
        c_copy(0, R_C, t).start()
        for j in range(H // 2):
            for p, w in enumerate(_head_pair(wuk_u32, t, j)):
                rows = pl.ds((2 * j + p) * B, B)
                q = q_s[rows, :].astype(BF16)
                qabs_s[t, rows, :] = lax.dot_general(q, w, NT, preferred_element_type=F32)
        return _
    lax.fori_loop(0, 4, qabs_step, None)

    def c_round(b, _):
        r = R_C + b
        qa = jnp.concatenate(
            [qabs_s[i, pl.ds(b, H, stride=B), :] for i in range(DC // 128)], axis=1
        ).astype(BF16)
        for t in range(4):
            c_copy(b, r, t).wait()

            @pl.when(b < B - 1)
            def _():
                c_copy(b + 1, r + 1, t).start()

            @pl.when(b == B - 1)
            def _():
                cp_bwq(t).start()

            c = c_v[r % 2, pl.ds(t * CK, CK), :]
            s = lax.dot_general(qa, c, NT, preferred_element_type=F32) * (D ** -0.5 * LOG2E)
            m_blk = s.max(axis=1, keepdims=True)
            if t == 0:
                m = m_blk
                p = jnp.exp2(s - m)
                l = p.sum(axis=1, keepdims=True)
                acc = jnp.dot(p.astype(BF16), c, preferred_element_type=F32)
            else:
                m_new = jnp.maximum(m, m_blk)
                alpha = jnp.exp2(m - m_new)
                p = jnp.exp2(s - m_new)
                l = alpha * l + p.sum(axis=1, keepdims=True)
                acc = alpha * acc + jnp.dot(p.astype(BF16), c, preferred_element_type=F32)
                m = m_new
        ctx = acc / l
        for i in range(DC // 128):
            ctxc_s[i, pl.ds(b, H, stride=B), :] = ctx[:, i * 128:(i + 1) * 128]
        return _
    lax.fori_loop(0, B, c_round, None)

    qb = None
    for t in range(4):
        cp_bwq(t).wait()
        cp_wuv(t).start()
        part = jnp.dot(x_s[t].astype(BF16), bwq_v[pl.ds(t * 128, 128), :], preferred_element_type=F32)
        qb = part if qb is None else qb + part
    for h in range(H):
        qb_s[pl.ds(h * B, B), :] = qb[:, h * D:(h + 1) * D]

    def ctx_step(t, _):
        cp_wuv(t).wait()
        for u in range(4):
            @pl.when(t == u)
            def _():
                kv_copy(0, R_KV, u).start()
        for j in range(H // 2):
            for p, w in enumerate(_head_pair(wuv_u32, t, j)):
                rows = pl.ds((2 * j + p) * B, B)
                cc = ctxc_s[t, rows, :].astype(BF16)
                ctx_s[rows, :] += jnp.dot(cc, w, preferred_element_type=F32)
        return _
    lax.fori_loop(0, 4, ctx_step, None)

    def kv_round(b, _):
        r = R_KV + b
        for half in range(2):
            for t in (2 * half, 2 * half + 1):
                kv_copy(b, r, t).wait()

                @pl.when(b < B - 1)
                def _():
                    kv_copy(b + 1, r + 1, t).start()

                @pl.when(b == B - 1)
                def _():
                    cp_wo(t).start()

            for i in (2 * half, 2 * half + 1):
                q8 = qb_s[pl.ds(b + 8 * i * B, 8, stride=B), :].astype(BF16)
                first = lax.broadcasted_iota(jnp.int32, (8, 1), 0) < 4
                s0 = lax.dot_general(q8, k_v[r % 2, 2 * i], NT, preferred_element_type=F32)
                s1 = lax.dot_general(q8, k_v[r % 2, 2 * i + 1], NT, preferred_element_type=F32)
                s = jnp.where(first, s0, s1) * (D ** -0.5 * LOG2E)
                p = jnp.exp2(s - s.max(axis=1, keepdims=True))
                l = p.sum(axis=1, keepdims=True)
                pb = p.astype(BF16)
                o0 = jnp.dot(pb, v_v[r % 2, 2 * i], preferred_element_type=F32)
                o1 = jnp.dot(pb, v_v[r % 2, 2 * i + 1], preferred_element_type=F32)
                ob_s[pl.ds(b + 8 * i * B, 8, stride=B), :] = jnp.where(first, o0, o1) / l
        return _
    lax.fori_loop(0, B, kv_round, None)

    gw_cp.wait()
    gate = jax.nn.sigmoid(
        (x.astype(F32) * gw_v[...].astype(F32).reshape(1, M)).sum(axis=1, keepdims=True))

    def lhs(scratch, t):
        return jnp.concatenate(
            [scratch[pl.ds((8 * t + h) * B, B), :] for h in range(8)], axis=1).astype(BF16)

    out_a = jnp.zeros((B, M), F32)
    for t in range(4):
        cp_wo(t).wait()
        cp_bwo(t).start()
        out_a += jnp.dot(lhs(ctx_s, t), wo_v[pl.ds(t * 1024, 1024), :], preferred_element_type=F32)
    out = gate * out_a
    for t in range(4):
        ob = lhs(ob_s, t)
        cp_bwo(t).wait()
        out_b = jnp.dot(ob, bwo_v[pl.ds(t * 1024, 1024), :], preferred_element_type=F32)
        out += (1.0 - gate) * out_b
    o_ref[...] = out.astype(o_ref.dtype)


@jax.jit
def pallas_gated_mix__compressed_kv_cla__sliding_block_cached__decode_kernel(
    A_x: jax.Array,
    A_c_kv: jax.Array,
    A_w_q: jax.Array,
    A_w_uk: jax.Array,
    A_w_uv: jax.Array,
    A_w_o: jax.Array,
    B_x: jax.Array,
    B_k_cache: jax.Array,
    B_v_cache: jax.Array,
    B_wq: jax.Array,
    B_wo: jax.Array,
    gate_w: jax.Array,
):
    del B_x
    hbm = pl.BlockSpec(memory_space=pl.ANY)
    rows_bh = B * H
    out = pl.pallas_call(
        _kernel,
        out_shape=jax.ShapeDtypeStruct((B, M), BF16),
        in_specs=[hbm] * 11,
        out_specs=pl.BlockSpec(memory_space=pltpu.VMEM),
        scratch_shapes=[
            pltpu.VMEM((B, M), BF16),
            pltpu.VMEM((M,), BF16),
            pltpu.VMEM((M * H // 2, D), jnp.uint32),
            pltpu.VMEM((DC * H // 2, D), jnp.uint32),
            pltpu.VMEM((DC * H // 2, D), jnp.uint32),
            pltpu.VMEM((H * D, M), BF16),
            pltpu.VMEM((M, H * D), BF16),
            pltpu.VMEM((H * D, M), BF16),
            pltpu.VMEM((2, SK, DC), BF16),
            pltpu.VMEM((2, HKV, WIN, D), BF16),
            pltpu.VMEM((2, HKV, WIN, D), BF16),
            pltpu.VMEM((4, B, 128), F32),
            pltpu.VMEM((rows_bh, D), F32),
            pltpu.VMEM((rows_bh, D), F32),
            pltpu.VMEM((DC // 128, rows_bh, 128), F32),
            pltpu.VMEM((rows_bh, D), F32),
            pltpu.VMEM((DC // 128, rows_bh, 128), F32),
            pltpu.VMEM((rows_bh, D), F32),
            pltpu.SemaphoreType.DMA((2, 4)),
            pltpu.SemaphoreType.DMA((2,)),
        ],
        compiler_params=pltpu.CompilerParams(vmem_limit_bytes=64 * 1024 * 1024),
    )(
        A_x.reshape(B, M), gate_w, A_c_kv,
        A_w_q.reshape(M * H, D), A_w_uk.reshape(DC * H, D), A_w_uv.reshape(DC * H, D),
        A_w_o.reshape(H * D, M), B_k_cache, B_v_cache, B_wq, B_wo,
    )
    return out.reshape(B, 1, M)
```

```python
import math

import jax
import jax.numpy as jnp
from jax import lax
import jax.experimental.pallas as pl
import jax.experimental.pallas.tpu as pltpu

B = 8
H = 32
D = 128
M = 512
DC = 512
SK = 4096
HKV = 8
WIN = 1024
CK = SK // 4
SCALE = D ** -0.5 * math.log2(math.e)

F32 = jnp.float32
BF16 = jnp.bfloat16
NT = (((1,), (1,)), ((), ()))

PIECE_BYTES = 32 * 1024
N_SEMS = 5
R_WQ, R_WUK, R_C, R_BWQ, R_WUV, R_KV, R_WO, R_BWO = 0, 1, 2, 10, 11, 12, 20, 21


class _Chunk:
    def __init__(self, src, dst, sem, pieces):
        self.src, self.dst, self.sem, self.pieces = src, dst, sem, pieces

    def start(self):
        half = len(self.pieces) // 2
        for i in range(half):
            for queue in range(2):
                idx = self.pieces[queue * half + i]
                pltpu.make_async_copy(self.src.at[idx], self.dst.at[idx], self.sem).start(
                    priority=queue)

    def wait(self):
        pltpu.make_async_copy(self.dst, self.dst, self.sem).wait()


def _row_pieces(rows, cols):
    n = PIECE_BYTES // (2 * cols)
    return [(pl.ds(i * n, n),) for i in range(rows // n)]


def _tile_pieces(rows, cols):
    n = PIECE_BYTES // (2 * 8)
    return [(pl.ds(i * 8, 8), pl.ds(j * n, n)) for i in range(rows // 8) for j in range(cols // n)]


def _head_pair(w_u32, t, j):
    w = w_u32[pl.ds(t * (128 * H // 2) + j, 128, stride=H // 2), :]
    lo = pltpu.bitcast(w << 16, F32).astype(BF16)
    hi = pltpu.bitcast(w & jnp.uint32(0xFFFF0000), F32).astype(BF16)
    return lo, hi


def _kernel(x_hbm, gw_hbm, c_hbm, wq_hbm, wuk_hbm, wuv_hbm, wo_hbm, k_hbm, v_hbm,
            bwq_hbm, bwo_hbm, o_ref,
            x_v, gw_v, wq_u32, wuk_u32, wuv_u32, wo_v, bwq_v, bwo_v, c_v, k_v, v_v,
            x_s, q_s, ctx_s, qabs_s, qb_s, ctxc_s, ob_s, sems):

    def sem(r, t):
        return sems.at[(4 * r + t) % N_SEMS]

    def weight_chunk(src, dst, rows, cols, r, t):
        n = rows // 4
        pieces = _tile_pieces(n, cols) if 16 * cols > PIECE_BYTES else _row_pieces(n, cols)
        return _Chunk(src.at[pl.ds(t * n, n)], dst.at[pl.ds(t * n, n)], sem(r, t), pieces)

    def c_chunk(b, r, t):
        rows = pl.ds(t * CK, CK)
        return _Chunk(c_hbm.at[b, rows], c_v.at[r % 2, rows], sem(r, t), _row_pieces(CK, DC))

    def kv_chunk(b, r, t):
        src, dst = (k_hbm, k_v) if t % 2 == 0 else (v_hbm, v_v)
        heads = pl.ds((t // 2) * (HKV // 2), HKV // 2)
        pieces = [(g,) + rows for g in range(HKV // 2) for rows in _row_pieces(WIN, D)]
        return _Chunk(src.at[b, heads, pl.ds(SK - WIN, WIN)], dst.at[r % 2, heads],
                      sem(r, t), pieces)

    wq_chunk = lambda t: weight_chunk(wq_hbm, wq_u32.bitcast(BF16), M * H, D, R_WQ, t)
    wuk_chunk = lambda t: weight_chunk(wuk_hbm, wuk_u32.bitcast(BF16), DC * H, D, R_WUK, t)
    wuv_chunk = lambda t: weight_chunk(wuv_hbm, wuv_u32.bitcast(BF16), DC * H, D, R_WUV, t)
    bwq_chunk = lambda t: weight_chunk(bwq_hbm, bwq_v, M, H * D, R_BWQ, t)
    wo_chunk = lambda t: weight_chunk(wo_hbm, wo_v, H * D, M, R_WO, t)
    bwo_chunk = lambda t: weight_chunk(bwo_hbm, bwo_v, H * D, M, R_BWO, t)

    def last_chunk_part(i):
        rows = pl.ds(3072 + i * 512, 512)
        return _Chunk(bwo_hbm.at[rows], bwo_v.at[rows], (sem(R_WO, 3), sem(R_BWO, 3))[i],
                      _row_pieces(512, M))

    x_copy = pltpu.make_async_copy(x_hbm, x_v, sem(R_WUK, 0))
    gw_copy = pltpu.make_async_copy(gw_hbm, gw_v, sem(R_WUK, 0))
    wq_chunk(0).start()
    x_copy.start()
    gw_copy.start()
    for t in range(1, 4):
        wq_chunk(t).start()
    x_copy.wait()
    gw_copy.wait()

    x = x_v[...].astype(F32)
    gate = jax.nn.sigmoid(
        (x * gw_v[...].astype(F32).reshape(1, M)).sum(axis=1, keepdims=True))
    for t in range(4):
        x_s[t] = x[:, t * 128:(t + 1) * 128]
    q_s[...] = jnp.zeros_like(q_s)
    ctx_s[...] = jnp.zeros_like(ctx_s)

    def q_step(t, carry):
        wq_chunk(t).wait()
        wuk_chunk(t).start()
        xt = x_s[t].astype(BF16)
        for j in range(H // 2):
            for p, w in enumerate(_head_pair(wq_u32, t, j)):
                rows = pl.ds((2 * j + p) * B, B)
                q_s[rows, :] += jnp.dot(xt, w, preferred_element_type=F32)
        return carry
    lax.fori_loop(0, 4, q_step, None)

    def absorb_step(t, carry):
        wuk_chunk(t).wait()
        c_chunk(0, R_C, t).start()
        for j in range(H // 2):
            for p, w in enumerate(_head_pair(wuk_u32, t, j)):
                rows = pl.ds((2 * j + p) * B, B)
                q = q_s[rows, :].astype(BF16)
                qabs_s[t, rows, :] = lax.dot_general(q, w, NT, preferred_element_type=F32)
        return carry
    lax.fori_loop(0, 4, absorb_step, None)

    def c_round(b, carry):
        r = R_C + b
        qa = jnp.concatenate(
            [qabs_s[i, pl.ds(b, H, stride=B), :] for i in range(DC // 128)], axis=1
        ).astype(BF16)
        for t in range(4):
            c_chunk(b, r, t).wait()

            @pl.when(b < B - 1)
            def _():
                c_chunk(b + 1, r + 1, t).start()

            @pl.when(b == B - 1)
            def _():
                bwq_chunk(t).start()

            c = c_v[r % 2, pl.ds(t * CK, CK), :]
            s = lax.dot_general(qa, c, NT, preferred_element_type=F32) * SCALE
            m_blk = s.max(axis=1, keepdims=True)
            if t == 0:
                m = m_blk
                p = jnp.exp2(s - m)
                l = p.sum(axis=1, keepdims=True)
                acc = jnp.dot(p.astype(BF16), c, preferred_element_type=F32)
            else:
                m_new = jnp.maximum(m, m_blk)
                alpha = jnp.exp2(m - m_new)
                p = jnp.exp2(s - m_new)
                l = alpha * l + p.sum(axis=1, keepdims=True)
                acc = alpha * acc + jnp.dot(p.astype(BF16), c, preferred_element_type=F32)
                m = m_new
        ctx = acc / l
        for i in range(DC // 128):
            ctxc_s[i, pl.ds(b, H, stride=B), :] = ctx[:, i * 128:(i + 1) * 128]
        return carry
    lax.fori_loop(0, B, c_round, None)

    qb = None
    for t in range(4):
        bwq_chunk(t).wait()
        wuv_chunk(t).start()
        part = jnp.dot(x_s[t].astype(BF16), bwq_v[pl.ds(t * 128, 128), :],
                       preferred_element_type=F32)
        qb = part if qb is None else qb + part
    for h in range(H):
        qb_s[pl.ds(h * B, B), :] = qb[:, h * D:(h + 1) * D]

    def ctx_step(t, carry):
        wuv_chunk(t).wait()
        for u in range(4):
            @pl.when(t == u)
            def _():
                kv_chunk(0, R_KV, u).start()

        for j in range(H // 2):
            for p, w in enumerate(_head_pair(wuv_u32, t, j)):
                rows = pl.ds((2 * j + p) * B, B)
                cc = ctxc_s[t, rows, :].astype(BF16)
                ctx_s[rows, :] += jnp.dot(cc, w, preferred_element_type=F32)
        return carry
    lax.fori_loop(0, 4, ctx_step, None)

    def kv_round(b, carry):
        r = R_KV + b
        first = lax.broadcasted_iota(jnp.int32, (8, 1), 0) < 4
        for half in range(2):
            for t in (2 * half, 2 * half + 1):
                kv_chunk(b, r, t).wait()

                @pl.when(b < B - 1)
                def _():
                    kv_chunk(b + 1, r + 1, t).start()

                @pl.when(b == B - 1)
                def _():
                    wo_chunk(t).start()

            for i in (2 * half, 2 * half + 1):
                heads = pl.ds(b + 8 * i * B, 8, stride=B)
                q8 = qb_s[heads, :].astype(BF16)
                s0 = lax.dot_general(q8, k_v[r % 2, 2 * i], NT, preferred_element_type=F32)
                s1 = lax.dot_general(q8, k_v[r % 2, 2 * i + 1], NT, preferred_element_type=F32)
                s = jnp.where(first, s0, s1) * SCALE
                p = jnp.exp2(s - s.max(axis=1, keepdims=True))
                l = p.sum(axis=1, keepdims=True)
                p = p.astype(BF16)
                o0 = jnp.dot(p, v_v[r % 2, 2 * i], preferred_element_type=F32)
                o1 = jnp.dot(p, v_v[r % 2, 2 * i + 1], preferred_element_type=F32)
                ob_s[heads, :] = jnp.where(first, o0, o1) / l
        return carry
    lax.fori_loop(0, B, kv_round, None)

    def heads_side_by_side(scratch, h0, n):
        return jnp.concatenate(
            [scratch[pl.ds(h * B, B), :] for h in range(h0, h0 + n)], axis=1).astype(BF16)

    out_a = jnp.zeros((B, M), F32)
    for t in range(4):
        wo_chunk(t).wait()
        if t < 3:
            bwo_chunk(t).start()
        else:
            last_chunk_part(0).start()
            last_chunk_part(1).start()
        out_a += jnp.dot(heads_side_by_side(ctx_s, 8 * t, 8), wo_v[pl.ds(t * 1024, 1024), :],
                         preferred_element_type=F32)

    out_b = jnp.zeros((B, M), F32)
    for t in range(3):
        ob = heads_side_by_side(ob_s, 8 * t, 8)
        bwo_chunk(t).wait()
        out_b += jnp.dot(ob, bwo_v[pl.ds(t * 1024, 1024), :], preferred_element_type=F32)
    for i in range(2):
        ob = heads_side_by_side(ob_s, 24 + 4 * i, 4)
        last_chunk_part(i).wait()
        out_b += jnp.dot(ob, bwo_v[pl.ds(3072 + i * 512, 512), :], preferred_element_type=F32)

    o_ref[...] = (gate * out_a + (1.0 - gate) * out_b).astype(o_ref.dtype)


@jax.jit
def pallas_gated_mix__compressed_kv_cla__sliding_block_cached__decode_kernel(
    A_x: jax.Array,
    A_c_kv: jax.Array,
    A_w_q: jax.Array,
    A_w_uk: jax.Array,
    A_w_uv: jax.Array,
    A_w_o: jax.Array,
    B_x: jax.Array,
    B_k_cache: jax.Array,
    B_v_cache: jax.Array,
    B_wq: jax.Array,
    B_wo: jax.Array,
    gate_w: jax.Array,
):
    del B_x
    out = pl.pallas_call(
        _kernel,
        out_shape=jax.ShapeDtypeStruct((B, M), BF16),
        in_specs=[pl.BlockSpec(memory_space=pl.ANY)] * 11,
        out_specs=pl.BlockSpec(memory_space=pltpu.VMEM),
        scratch_shapes=[
            pltpu.VMEM((B, M), BF16),
            pltpu.VMEM((M,), BF16),
            pltpu.VMEM((M * H // 2, D), jnp.uint32),
            pltpu.VMEM((DC * H // 2, D), jnp.uint32),
            pltpu.VMEM((DC * H // 2, D), jnp.uint32),
            pltpu.VMEM((H * D, M), BF16),
            pltpu.VMEM((M, H * D), BF16),
            pltpu.VMEM((H * D, M), BF16),
            pltpu.VMEM((2, SK, DC), BF16),
            pltpu.VMEM((2, HKV, WIN, D), BF16),
            pltpu.VMEM((2, HKV, WIN, D), BF16),
            pltpu.VMEM((M // 128, B, 128), F32),
            pltpu.VMEM((H * B, D), F32),
            pltpu.VMEM((H * B, D), F32),
            pltpu.VMEM((DC // 128, H * B, 128), F32),
            pltpu.VMEM((H * B, D), F32),
            pltpu.VMEM((DC // 128, H * B, 128), F32),
            pltpu.VMEM((H * B, D), F32),
            pltpu.SemaphoreType.DMA((N_SEMS,)),
        ],
        compiler_params=pltpu.CompilerParams(vmem_limit_bytes=64 * 1024 * 1024),
    )(
        A_x.reshape(B, M), gate_w, A_c_kv,
        A_w_q.reshape(M * H, D), A_w_uk.reshape(DC * H, D), A_w_uv.reshape(DC * H, D),
        A_w_o.reshape(H * D, M), B_k_cache, B_v_cache, B_wq, B_wo,
    )
    return out.reshape(B, 1, M)
```

```python
import math

import jax
import jax.numpy as jnp
from jax import lax
import jax.experimental.pallas as pl
import jax.experimental.pallas.tpu as pltpu

B = 8
H = 32
D = 128
M = 512
DC = 512
SK = 4096
HKV = 8
WIN = 1024
CK = SK // 4
SCALE = D ** -0.5 * math.log2(math.e)

F32 = jnp.float32
BF16 = jnp.bfloat16
NT = (((1,), (1,)), ((), ()))

PIECE_BYTES = 32 * 1024
TR_PITCH = 129
N_SEMS = 5
R_WQ, R_WUK, R_C, R_BWQ, R_WUV, R_KV, R_WO, R_BWO = 0, 1, 2, 10, 11, 12, 20, 21


class _Chunk:
    def __init__(self, src, dst, sem, pieces):
        self.src, self.dst, self.sem, self.pieces = src, dst, sem, pieces

    def start(self):
        half = len(self.pieces) // 2
        for i in range(half):
            for queue in range(2):
                idx = self.pieces[queue * half + i]
                pltpu.make_async_copy(self.src.at[idx], self.dst.at[idx], self.sem).start(
                    priority=queue)

    def wait(self):
        pltpu.make_async_copy(self.dst, self.dst, self.sem).wait()


def _row_pieces(rows, cols):
    n = PIECE_BYTES // (2 * cols)
    return [(pl.ds(i * n, n),) for i in range(rows // n)]


def _tile_pieces(rows, cols):
    n = PIECE_BYTES // (2 * 8)
    return [(pl.ds(i * 8, 8), pl.ds(j * n, n)) for i in range(rows // 8) for j in range(cols // n)]


def _split_heads(w_v, tr_s, t):
    base = pl.multiple_of(t * (128 * H), 128 * H)
    for i in range(128):
        words = pltpu.bitcast(w_v[pl.ds(base + i * H, H), :], jnp.uint32)
        tr_s[pl.ds(i, H // 2, stride=TR_PITCH), :] = words
    heads = []
    for j in range(H // 2):
        w = tr_s[pl.ds(j * TR_PITCH, 128), :]
        heads.append(pltpu.bitcast(w << 16, F32).astype(BF16))
        heads.append(pltpu.bitcast(w & jnp.uint32(0xFFFF0000), F32).astype(BF16))
    return heads


def _kernel(x_hbm, gw_hbm, c_hbm, wq_hbm, wuk_hbm, wuv_hbm, wo_hbm, k_hbm, v_hbm,
            bwq_hbm, bwo_hbm, o_ref,
            x_v, gw_v, wq_v, wuk_v, wuv_v, wo_v, bwq_v, bwo_v, c_v, k_v, v_v,
            x_s, tr_s, q_s, ctx_s, qabs_s, qb_s, ctxc_s, ob_s, sems):

    def sem(r, t):
        return sems.at[(4 * r + t) % N_SEMS]

    def weight_chunk(src, dst, rows, cols, r, t):
        n = rows // 4
        pieces = _tile_pieces(n, cols) if 16 * cols > PIECE_BYTES else _row_pieces(n, cols)
        return _Chunk(src.at[pl.ds(t * n, n)], dst.at[pl.ds(t * n, n)], sem(r, t), pieces)

    def c_chunk(b, r, t):
        rows = pl.ds(t * CK, CK)
        return _Chunk(c_hbm.at[b, rows], c_v.at[r % 2, rows], sem(r, t), _row_pieces(CK, DC))

    def kv_chunk(b, r, t):
        src, dst = (k_hbm, k_v) if t % 2 == 0 else (v_hbm, v_v)
        heads = pl.ds((t // 2) * (HKV // 2), HKV // 2)
        pieces = [(g,) + rows for g in range(HKV // 2) for rows in _row_pieces(WIN, D)]
        return _Chunk(src.at[b, heads, pl.ds(SK - WIN, WIN)], dst.at[r % 2, heads],
                      sem(r, t), pieces)

    wq_chunk = lambda t: weight_chunk(wq_hbm, wq_v, M * H, D, R_WQ, t)
    wuk_chunk = lambda t: weight_chunk(wuk_hbm, wuk_v, DC * H, D, R_WUK, t)
    wuv_chunk = lambda t: weight_chunk(wuv_hbm, wuv_v, DC * H, D, R_WUV, t)
    bwq_chunk = lambda t: weight_chunk(bwq_hbm, bwq_v, M, H * D, R_BWQ, t)
    wo_chunk = lambda t: weight_chunk(wo_hbm, wo_v, H * D, M, R_WO, t)
    bwo_chunk = lambda t: weight_chunk(bwo_hbm, bwo_v, H * D, M, R_BWO, t)

    def last_chunk_part(i):
        rows = pl.ds(3072 + i * 512, 512)
        return _Chunk(bwo_hbm.at[rows], bwo_v.at[rows], (sem(R_WO, 3), sem(R_BWO, 3))[i],
                      _row_pieces(512, M))

    x_copy = pltpu.make_async_copy(x_hbm, x_v, sem(R_WUK, 0))
    gw_copy = pltpu.make_async_copy(gw_hbm, gw_v, sem(R_WUK, 0))
    wq_chunk(0).start()
    x_copy.start()
    gw_copy.start()
    for t in range(1, 4):
        wq_chunk(t).start()
    x_copy.wait()
    gw_copy.wait()

    x = x_v[...].astype(F32)
    gate = jax.nn.sigmoid(
        (x * gw_v[...].astype(F32).reshape(1, M)).sum(axis=1, keepdims=True))
    for t in range(4):
        x_s[t] = x[:, t * 128:(t + 1) * 128]
    q_s[...] = jnp.zeros_like(q_s)
    ctx_s[...] = jnp.zeros_like(ctx_s)

    def q_step(t, carry):
        wq_chunk(t).wait()
        wuk_chunk(t).start()
        xt = x_s[t].astype(BF16)
        for h, w in enumerate(_split_heads(wq_v, tr_s, t)):
            rows = pl.ds(h * B, B)
            q_s[rows, :] += jnp.dot(xt, w, preferred_element_type=F32)
        return carry
    lax.fori_loop(0, 4, q_step, None)

    def absorb_step(t, carry):
        wuk_chunk(t).wait()
        c_chunk(0, R_C, t).start()
        for h, w in enumerate(_split_heads(wuk_v, tr_s, t)):
            rows = pl.ds(h * B, B)
            q = q_s[rows, :].astype(BF16)
            qabs_s[t, rows, :] = lax.dot_general(q, w, NT, preferred_element_type=F32)
        return carry
    lax.fori_loop(0, 4, absorb_step, None)

    def c_round(b, carry):
        r = R_C + b
        qa = jnp.concatenate(
            [qabs_s[i, pl.ds(b, H, stride=B), :] for i in range(DC // 128)], axis=1
        ).astype(BF16)
        for t in range(4):
            c_chunk(b, r, t).wait()

            @pl.when(b < B - 1)
            def _():
                c_chunk(b + 1, r + 1, t).start()

            @pl.when(b == B - 1)
            def _():
                bwq_chunk(t).start()

            c = c_v[r % 2, pl.ds(t * CK, CK), :]
            s = lax.dot_general(qa, c, NT, preferred_element_type=F32) * SCALE
            m_blk = s.max(axis=1, keepdims=True)
            if t == 0:
                m = m_blk
                p = jnp.exp2(s - m)
                l = p.sum(axis=1, keepdims=True)
                acc = jnp.dot(p.astype(BF16), c, preferred_element_type=F32)
            else:
                m_new = jnp.maximum(m, m_blk)
                alpha = jnp.exp2(m - m_new)
                p = jnp.exp2(s - m_new)
                l = alpha * l + p.sum(axis=1, keepdims=True)
                acc = alpha * acc + jnp.dot(p.astype(BF16), c, preferred_element_type=F32)
                m = m_new
        ctx = acc / l
        for i in range(DC // 128):
            ctxc_s[i, pl.ds(b, H, stride=B), :] = ctx[:, i * 128:(i + 1) * 128]
        return carry
    lax.fori_loop(0, B, c_round, None)

    qb = None
    for t in range(4):
        bwq_chunk(t).wait()
        wuv_chunk(t).start()
        part = jnp.dot(x_s[t].astype(BF16), bwq_v[pl.ds(t * 128, 128), :],
                       preferred_element_type=F32)
        qb = part if qb is None else qb + part
    for h in range(H):
        qb_s[pl.ds(h * B, B), :] = qb[:, h * D:(h + 1) * D]

    def ctx_step(t, carry):
        wuv_chunk(t).wait()
        for u in range(4):
            @pl.when(t == u)
            def _():
                kv_chunk(0, R_KV, u).start()

        for h, w in enumerate(_split_heads(wuv_v, tr_s, t)):
            rows = pl.ds(h * B, B)
            cc = ctxc_s[t, rows, :].astype(BF16)
            ctx_s[rows, :] += jnp.dot(cc, w, preferred_element_type=F32)
        return carry
    lax.fori_loop(0, 4, ctx_step, None)

    def kv_round(b, carry):
        r = R_KV + b
        first = lax.broadcasted_iota(jnp.int32, (8, 1), 0) < 4
        for half in range(2):
            for t in (2 * half, 2 * half + 1):
                kv_chunk(b, r, t).wait()

                @pl.when(b < B - 1)
                def _():
                    kv_chunk(b + 1, r + 1, t).start()

                @pl.when(b == B - 1)
                def _():
                    wo_chunk(t).start()

            for i in (2 * half, 2 * half + 1):
                heads = pl.ds(b + 8 * i * B, 8, stride=B)
                q8 = qb_s[heads, :].astype(BF16)
                s0 = lax.dot_general(q8, k_v[r % 2, 2 * i], NT, preferred_element_type=F32)
                s1 = lax.dot_general(q8, k_v[r % 2, 2 * i + 1], NT, preferred_element_type=F32)
                s = jnp.where(first, s0, s1) * SCALE
                p = jnp.exp2(s - s.max(axis=1, keepdims=True))
                l = p.sum(axis=1, keepdims=True)
                p = p.astype(BF16)
                o0 = jnp.dot(p, v_v[r % 2, 2 * i], preferred_element_type=F32)
                o1 = jnp.dot(p, v_v[r % 2, 2 * i + 1], preferred_element_type=F32)
                ob_s[heads, :] = jnp.where(first, o0, o1) / l
        return carry
    lax.fori_loop(0, B, kv_round, None)

    def heads_side_by_side(scratch, h0, n):
        return jnp.concatenate(
            [scratch[pl.ds(h * B, B), :] for h in range(h0, h0 + n)], axis=1).astype(BF16)

    out_a = jnp.zeros((B, M), F32)
    for t in range(4):
        wo_chunk(t).wait()
        if t < 3:
            bwo_chunk(t).start()
        else:
            last_chunk_part(0).start()
            last_chunk_part(1).start()
        out_a += jnp.dot(heads_side_by_side(ctx_s, 8 * t, 8), wo_v[pl.ds(t * 1024, 1024), :],
                         preferred_element_type=F32)

    out_b = jnp.zeros((B, M), F32)
    for t in range(3):
        ob = heads_side_by_side(ob_s, 8 * t, 8)
        bwo_chunk(t).wait()
        out_b += jnp.dot(ob, bwo_v[pl.ds(t * 1024, 1024), :], preferred_element_type=F32)
    for i in range(2):
        ob = heads_side_by_side(ob_s, 24 + 4 * i, 4)
        last_chunk_part(i).wait()
        out_b += jnp.dot(ob, bwo_v[pl.ds(3072 + i * 512, 512), :], preferred_element_type=F32)

    o_ref[...] = (gate * out_a + (1.0 - gate) * out_b).astype(o_ref.dtype)


@jax.jit
def pallas_gated_mix__compressed_kv_cla__sliding_block_cached__decode_kernel(
    A_x: jax.Array,
    A_c_kv: jax.Array,
    A_w_q: jax.Array,
    A_w_uk: jax.Array,
    A_w_uv: jax.Array,
    A_w_o: jax.Array,
    B_x: jax.Array,
    B_k_cache: jax.Array,
    B_v_cache: jax.Array,
    B_wq: jax.Array,
    B_wo: jax.Array,
    gate_w: jax.Array,
):
    del B_x
    out = pl.pallas_call(
        _kernel,
        out_shape=jax.ShapeDtypeStruct((B, M), BF16),
        in_specs=[pl.BlockSpec(memory_space=pl.ANY)] * 11,
        out_specs=pl.BlockSpec(memory_space=pltpu.VMEM),
        scratch_shapes=[
            pltpu.VMEM((B, M), BF16),
            pltpu.VMEM((M,), BF16),
            pltpu.VMEM((M * H, D), BF16),
            pltpu.VMEM((DC * H, D), BF16),
            pltpu.VMEM((DC * H, D), BF16),
            pltpu.VMEM((H * D, M), BF16),
            pltpu.VMEM((M, H * D), BF16),
            pltpu.VMEM((H * D, M), BF16),
            pltpu.VMEM((2, SK, DC), BF16),
            pltpu.VMEM((2, HKV, WIN, D), BF16),
            pltpu.VMEM((2, HKV, WIN, D), BF16),
            pltpu.VMEM((M // 128, B, 128), F32),
            pltpu.VMEM((H // 2 * TR_PITCH, D), jnp.uint32),
            pltpu.VMEM((H * B, D), F32),
            pltpu.VMEM((H * B, D), F32),
            pltpu.VMEM((DC // 128, H * B, 128), F32),
            pltpu.VMEM((H * B, D), F32),
            pltpu.VMEM((DC // 128, H * B, 128), F32),
            pltpu.VMEM((H * B, D), F32),
            pltpu.SemaphoreType.DMA((N_SEMS,)),
        ],
        compiler_params=pltpu.CompilerParams(vmem_limit_bytes=64 * 1024 * 1024),
    )(
        A_x.reshape(B, M), gate_w, A_c_kv,
        A_w_q.reshape(M * H, D), A_w_uk.reshape(DC * H, D), A_w_uv.reshape(DC * H, D),
        A_w_o.reshape(H * D, M), B_k_cache, B_v_cache, B_wq, B_wo,
    )
    return out.reshape(B, 1, M)
```
